```python
import os as _os
_os.environ.setdefault("JAX_PLATFORMS", "cpu")
import jax
import jax.numpy as jnp

def _softmax(x, axis=-1):
    return jax.nn.softmax(x, axis=axis)
def _gelu(x):
    return jax.nn.gelu(x, approximate=True)
def _silu(x):
    return jax.nn.silu(x)
def _sigmoid(x):
    return jax.nn.sigmoid(x)
def _layernorm(x, axis=-1, eps=1e-5):
    m = jnp.mean(x, axis=axis, keepdims=True)
    v = jnp.var(x, axis=axis, keepdims=True)
    return (x - m) / jnp.sqrt(v + eps)
def _scatter_add(tgt, idx, src, axis=0):
    return tgt.at[idx].add(src)
def _segment_sum(src, seg, n):
    return jax.ops.segment_sum(src, seg, n)
class _Rng:
    def __init__(self, key):
        self._k = key
    def _next(self):
        self._k, sub = jax.random.split(self._k)
        return sub
    def normal(self, shape):
        return jax.random.normal(self._next(), shape, dtype=jnp.bfloat16)
    def randint(self, lo, hi, shape):
        return jax.random.randint(self._next(), shape, lo, hi, dtype=jnp.int32)
    def uniform(self, shape, lo=0.0, hi=1.0):
        return jax.random.uniform(self._next(), shape, jnp.bfloat16, lo, hi)
    def permutation(self, n):
        return jax.random.permutation(self._next(), n)


kernel_name = 'parallel_sum__sliding_block__moe_arch_mod__prompt'

def setup_inputs():
    _rng = _Rng(jax.random.key(int.from_bytes(__import__("os").urandom(4), "little")))
    _w = (lambda a: (lambda t: t.astype(jnp.bfloat16) if jnp.issubdtype(t.dtype, jnp.floating) else t)(jnp.asarray(a)))
    def _A_setup():
        B, S, D = 1, 2048, 512
        return {
            "x": _w((lambda *s: _rng.normal(s) * 0.05)(B, S, D)),
            "wqkv": _w((lambda *s: _rng.normal(s) * 0.05)(D, 3 * D)),
            "wo": _w((lambda *s: _rng.normal(s) * 0.05)(D, D)),
        }
    _A_in = _A_setup()

    def _B_setup():
        B, S, D, F, C = 1, 2048, 512, 1376, 1
        return {
            "x": _w((lambda *s: _rng.normal(s) * 0.05)(B, S, D)),
            "w_r": _w((lambda *s: _rng.normal(s) * 0.05)(D)),
            "w_gate": _w((lambda *s: _rng.normal(s) * 0.05)(D, F)),
            "w_up": _w((lambda *s: _rng.normal(s) * 0.05)(D, F)),
            "w_down": _w((lambda *s: _rng.normal(s) * 0.05)(F, D)),
        }
    _B_in = _B_setup()

    return {
        "A_x": _A_in["x"],
        "A_wqkv": _A_in["wqkv"],
        "A_wo": _A_in["wo"],
        "B_x": _B_in["x"],
        "B_w_r": _B_in["w_r"],
        "B_w_gate": _B_in["w_gate"],
        "B_w_up": _B_in["w_up"],
        "B_w_down": _B_in["w_down"],
    }

def reference(A_x, A_wqkv, A_wo, B_x, B_w_r, B_w_gate, B_w_up, B_w_down):
    def _A_ref(x, wqkv, wo):
        B, S, D = x.shape
        H = 32; Dh = D // H; W = 256
        qkv = (lambda x, *d: x.transpose(*d))((x @ wqkv).reshape(B, S, 3, H, Dh), 2, 0, 3, 1, 4)
        q, k, v = qkv[0], qkv[1], qkv[2]
        scores = jnp.einsum("bhqd,bhkd->bhqk", q, k) * (Dh ** -0.5)
        idx = jnp.arange(S)
        mask = (idx[:, None] - idx[None, :] >= 0) & (idx[:, None] - idx[None, :] < W)
        scores = jnp.where(mask[None, None], scores, -1e9)
        p = _softmax(scores, axis=-1)
        o = jnp.einsum("bhqk,bhkd->bhqd", p, v)
        return (lambda x, *d: x.transpose(*d))(o, 0, 2, 1, 3).reshape(B, S, D) @ wo

    def _B_ref(x, w_r, w_gate, w_up, w_down):
        B, S, D = x.shape
        C = 1
        r = x @ w_r
        idx = jnp.argsort(-r, axis=-1)[:, :C]
        idx_e = jnp.repeat(idx.reshape(B, C, 1), D, axis=2)
        x_sel = jnp.take_along_axis(x, idx_e, axis=1)
        g = _silu(x_sel @ w_gate)
        u = x_sel @ w_up
        y = (g * u) @ w_down
        r_sel = _sigmoid(jnp.take_along_axis(r, idx, axis=1))
        y = y * r_sel.reshape(B, C, 1)
        b_off = (jnp.arange(B) * S).reshape(B, 1)
        flat_idx = (idx + b_off).reshape(B * C)
        zero = (x * 0.0).reshape(B * S, D)
        upd = _scatter_add(zero, flat_idx, y.reshape(B * C, D), axis=0)
        return x + upd.reshape(B, S, D)

    x = A_x
    xn = _layernorm(x, axis=-1)
    return x + _A_ref(xn, A_wqkv, A_wo) + _B_ref(xn, B_w_r, B_w_gate, B_w_up, B_w_down)
```

```python
import math

import jax
import jax.numpy as jnp
from jax import lax
from jax.experimental import pallas as pl
from jax.experimental.pallas import tpu as pltpu

bf16 = jnp.bfloat16
f32 = jnp.float32
i32 = jnp.int32

SEQ, D, DH, WIN, FF = 2048, 512, 16, 256, 1376
TB = 256
NA = SEQ // TB
LNCH = 16
QB = 128
NQ = SEQ // QB
PAD = 256
NEG = -1e9
QSCALE = DH ** -0.5 * math.log2(math.e)
NT = (SEQ + PAD) // 128
UNROLL_Q = 2
NT_DIMS = (((1,), (1,)), ((), ()))


def _rb(x):
    return x.astype(bf16).astype(f32)


def _kernel(x_hbm, wqkv_hbm, wo_hbm, wr_hbm, wg_hbm, wu_hbm, wd_hbm, out_hbm,
            x_v, wqkv_v, wo_v, wr_v, wg_v, wu_v, wd_v,
            xn_s, res_s, wr_s, q_s, k_s, vt_s, sa_s, sb_s, o_s, out_v,
            sem_x, sem_w, sem_m, sem_o):
    def x_copy(i):
        rows = pl.ds(i * TB, TB)
        return pltpu.make_async_copy(x_hbm.at[rows, :], x_v.at[rows, :], sem_x.at[i])

    def w_copy(g):
        cols = pl.ds(D * g, D)
        return pltpu.make_async_copy(wqkv_hbm.at[:, cols], wqkv_v.at[:, cols], sem_w.at[g])

    wq_copy, wk_copy, wv_copy = w_copy(0), w_copy(1), w_copy(2)
    wr_copy = pltpu.make_async_copy(wr_hbm, wr_v, sem_m.at[0])
    wo_copy = pltpu.make_async_copy(wo_hbm, wo_v, sem_m.at[1])
    ffn_copies = [pltpu.make_async_copy(wg_hbm, wg_v, sem_m.at[2]),
                  pltpu.make_async_copy(wu_hbm, wu_v, sem_m.at[3]),
                  pltpu.make_async_copy(wd_hbm, wd_v, sem_m.at[4])]
    x_copy(0).start()
    x_copy(1).start()
    wr_copy.start()
    wv_copy.start()

    k_s[pl.ds(0, PAD // 2), :] = jnp.zeros((PAD // 2, D), i32)
    vt_s[0] = jnp.zeros((256, 128), i32)
    vt_s[1] = jnp.zeros((256, 128), i32)

    row16 = lax.broadcasted_iota(i32, (16, 128), 0)

    def layer_norm(i, best, gate):
        wr = wr_s[...][0:1]
        z = None
        for c in range(TB // LNCH):
            r0 = pl.multiple_of(i * TB + LNCH * c, LNCH)
            xf = x_v[pl.ds(r0, LNCH), :].astype(f32)
            m32 = jnp.sum(xf, axis=-1, keepdims=True) * (1.0 / D)
            if z is not None:
                m32 = pltpu.bitcast(pltpu.bitcast(m32, i32) | z, f32)
            cen = xf - m32
            v32 = jnp.sum(cen * cen, axis=-1, keepdims=True) * (1.0 / D)
            d = _rb(xf - _rb(m32))
            ve = _rb(_rb(v32) + _rb(jnp.float32(1e-5)))
            s = _rb(ve * lax.rsqrt(ve))
            r = pltpu.reciprocal(s, approx=True)
            inv = r * (2.0 - s * r)
            if gate:
                z = lax.shift_right_logical(lax.shift_right_logical(pltpu.bitcast(inv, i32), 31), 1)
            xn = (d * inv).astype(bf16)
            xn32 = xn.astype(f32)
            xn_s[pl.ds(pl.multiple_of(r0 // 2, LNCH // 2), LNCH // 2), :] = pltpu.bitcast(xn, i32)
            res_s[pl.ds(r0, LNCH), :] = xf + xn32
            rr = _rb(jnp.sum(xn32 * wr, axis=-1, keepdims=True))
            rr = jnp.broadcast_to(jnp.where(rr != rr, -jnp.inf, rr), (LNCH, 128))
            upd = rr > best[0]
            best[0] = jnp.where(upd, rr, best[0])
            best[1] = jnp.where(upd, row16 + r0, best[1])
            yield

    def load_xn(i):
        return pltpu.bitcast(xn_s[pl.ds(pl.multiple_of(i * (TB // 2), TB // 2), TB // 2), :], bf16)

    def project(work, ln):
        def finish(i, j, d):
            r0 = pl.multiple_of(i * (TB // 2), TB // 2)
            cols = slice(128 * (j % 4), 128 * (j % 4) + 128)
            if j < 4:
                q_s[pl.ds(r0, TB // 2), cols] = pltpu.bitcast((d * QSCALE).astype(bf16), i32)
            elif j < 8:
                k_s[pl.ds(pl.multiple_of(r0 + PAD // 2, TB // 2), TB // 2), cols] = pltpu.bitcast(d.astype(bf16), i32)
            else:
                for t in range(TB // 128):
                    vt = d[128 * t:128 * t + 128].T.astype(bf16)
                    vt_s[i * (TB // 128) + PAD // 128 + t, pl.ds(64 * (j - 8), 64), :] = pltpu.bitcast(vt, i32)

        for i, xn, j in work:
            next(ln, None)
            finish(i, j, jnp.dot(xn, wqkv_v[:, 128 * j:128 * j + 128], preferred_element_type=f32))
        for _ in ln:
            pass

    V_COLS, K_COLS, Q_COLS = [8, 9, 10, 11], [4, 5, 6, 7], [0, 1, 2, 3]

    wr_copy.wait()
    wk_copy.start()
    wq_copy.start()
    x_copy(2).start()
    wr_s[...] = jnp.broadcast_to(wr_v[...].astype(f32).reshape(1, D), (8, D))
    best = [jnp.full((16, 128), -jnp.inf, f32), row16]
    for i in range(2):
        x_copy(i).wait()
        for _ in layer_norm(i, best, False):
            pass
    xn0, xn1 = load_xn(0), load_xn(1)
    wv_copy.wait()
    for i in range(3, NA):
        x_copy(i).start()
    project([(0, xn0, j) for j in V_COLS] + [(1, xn1, j) for j in V_COLS], iter(()))
    wk_copy.wait()
    wq_copy.wait()
    x_copy(2).wait()
    wo_copy.start()
    for c in ffn_copies:
        c.start()
    project([(0, xn0, j) for j in K_COLS + Q_COLS] + [(1, xn1, j) for j in K_COLS + Q_COLS],
            layer_norm(2, best, True))
    best = tuple(best)

    def phase_a(i, carry):
        best = list(carry[0])
        x_copy(i + 1).wait()
        xn = load_xn(i)
        project([(i, xn, j) for j in V_COLS + K_COLS + Q_COLS], layer_norm(i + 1, best, True))
        return tuple(best), (i >> 8)

    (best_v, best_i), zero = lax.fori_loop(2, NA - 1, phase_a, (best, 0))
    z0 = pl.multiple_of(zero * 8, 8)

    rmax = jnp.max(best_v, axis=0, keepdims=True)
    idx = jnp.min(jnp.where(best_v == rmax, best_i, SEQ), axis=0, keepdims=True)[0, 0]
    slab = pltpu.bitcast(xn_s[pl.ds(pl.multiple_of((idx >> 4) * 8, 8), 8), :], bf16).astype(f32)
    rowsel = lax.broadcasted_iota(i32, (16, D), 0) == (idx & 15)
    xsel = jnp.sum(jnp.where(rowsel, slab, 0.0), axis=0, keepdims=True)
    xsel16 = jnp.broadcast_to(xsel, (16, D)).astype(bf16)

    xn_last = load_xn(NA - 1)
    project([(NA - 1, xn_last, j) for j in V_COLS + K_COLS + Q_COLS], iter(()))

    for c in ffn_copies:
        c.wait()
    g = lax.dot_general(xsel16, wg_v[...], NT_DIMS, preferred_element_type=f32)
    u = lax.dot_general(xsel16, wu_v[...], NT_DIMS, preferred_element_type=f32)
    hmid = (g * jax.nn.sigmoid(g) * u).astype(bf16)
    y = jnp.dot(hmid, wd_v[...], preferred_element_type=f32)
    yrow = y[0:1] * jax.nn.sigmoid(rmax[:, 0:1])
    wo_copy.wait()

    lane = lax.broadcasted_iota(i32, (32, 128), 1)
    lane16i = lax.broadcasted_iota(i32, (16, 128), 1)
    col_j = lane16i & 63
    lane16 = lane16i < 64
    s_refs = [sa_s, sb_s]

    def first_chunk(static_a, ab):
        if static_a is None:
            return 0
        return max(0, PAD - (QB * static_a + 64 * ab)) // 16

    def qk(a, static_a, b, z0):
        hg, ab = b // 2, b % 2
        c0 = first_chunk(static_a, ab)
        qrow = pl.multiple_of(64 * a + 32 * ab, 32)
        qb = q_s[pl.ds(qrow, 32), 128 * hg:128 * hg + 128]
        parts = []
        for p in range(4):
            for hh in range(2):
                parts.append(jnp.where((lane >> 4) == 2 * p + (hh ^ ab), qb, 0))
        wt = pltpu.bitcast(jnp.concatenate(parts, axis=0), bf16)
        kw = pltpu.bitcast(k_s[pl.ds(pl.multiple_of(qrow + 8 * c0, 8), 160 - 8 * c0), 128 * hg:128 * hg + 128], bf16)
        st = lax.dot_general(kw, wt, NT_DIMS, preferred_element_type=f32)
        s_ref = s_refs[b % 2]
        acc = [None] * 4
        for c in range(c0, 20):
            for p in range(4):
                x = st[16 * (c - c0):16 * (c - c0) + 16, 128 * p:128 * p + 128]
                if c < 4:
                    x = jnp.where(row16 + 16 * c > col_j, x, NEG)
                elif c >= 16:
                    x = jnp.where(row16 + 16 * (c - 16) <= col_j, x, NEG)
                acc[p] = x if acc[p] is None else jnp.maximum(acc[p], x)
                s_ref[pl.ds(z0 + 16 * c, 16), 128 * p:128 * p + 128] = x
        for p in range(4):
            m = jnp.max(acc[p], axis=0, keepdims=True)
            s_ref[pl.ds(z0 + 320, 8), 128 * p:128 * p + 128] = jnp.broadcast_to(m, (8, 128))

    def sm_pv(a, static_a, b, z0):
        hg, ab = b // 2, b % 2
        c0 = first_chunk(static_a, ab)
        s_ref = s_refs[b % 2]
        m = [s_ref[pl.ds(z0 + 320, 8), 128 * p:128 * p + 128][0:1] for p in range(4)]
        chunks = [[] for _ in range(4)]
        acc = [None] * 4
        for c in range(c0, 20):
            for p in range(4):
                x = s_ref[pl.ds(z0 + 16 * c, 16), 128 * p:128 * p + 128]
                e = jnp.exp2(x - m[p])
                acc[p] = e if acc[p] is None else acc[p] + e
                chunks[p].append(e)
        lo = c0 + 4 * ab
        hi = 20 + 4 * ab
        t0 = lo // 8
        zero16 = jnp.zeros((16, 128), f32)
        res = []
        for p in range(4):
            l = jnp.sum(acc[p], axis=0, keepdims=True)
            rows = [zero16] * lo + chunks[p] + [zero16] * (24 - hi)
            ot = None
            for t in range(t0, 3):
                pt = jnp.concatenate(rows[8 * t:8 * t + 8], axis=0).astype(bf16)
                vv = pltpu.bitcast(vt_s[a + t, pl.ds(64 * hg + 16 * p, 16), :], bf16)
                d = jnp.dot(vv, pt, preferred_element_type=f32)
                ot = d if ot is None else ot + d
            rl = pltpu.reciprocal(l, approx=True)
            rl = rl * (2.0 - l * rl)
            res.append(ot * rl)
        return res

    def store_o(hg, held, r):
        rows = []
        for p in range(4):
            A, B = held[p], r[p]
            rows.append(jnp.where(lane16, A[0:16], B[0:16]))
            rows.append(jnp.where(lane16, B[16:32], A[16:32]))
        ot = jnp.concatenate(rows, axis=0)
        t = ot.T
        tsw = jnp.concatenate([t[64:128], t[0:64]], axis=0)
        odd = ((lax.broadcasted_iota(i32, (128, 128), 1) >> 4) & 1) == 1
        o = jnp.where(odd, tsw, t).astype(bf16)
        o_s[:, 128 * hg:128 * hg + 128] = pltpu.bitcast(o, i32)

    def out_copy(a):
        return pltpu.make_async_copy(out_v.at[a], out_hbm.at[pl.ds(pl.multiple_of(a * QB, QB), QB), :], sem_o.at[a])

    def out_proj(a, o):
        attn = jnp.dot(o, wo_v[...], preferred_element_type=f32)
        r0 = pl.multiple_of(a * QB, QB)
        rowid = lax.broadcasted_iota(i32, (QB, D), 0) + a * QB
        out = attn + res_s[pl.ds(r0, QB), :] + jnp.where(rowid == idx, yrow, 0.0)
        out_v[a] = out.astype(bf16)
        out_copy(a).start()

    def block(a, static_a, a_next, static_next, z0, do_out):
        if do_out:
            o_prev = pltpu.bitcast(o_s[...], bf16)
        held = None
        for b in range(8):
            if b < 7:
                qk(a, static_a, b + 1, z0)
            else:
                qk(a_next, static_next, 0, z0)
            r = sm_pv(a, static_a, b, z0)
            if b % 2 == 0:
                held = r
            else:
                store_o(b // 2, held, r)
        if do_out:
            out_proj(a - 1, o_prev)

    qk(0, 0, 0, z0)
    block(0, 0, 1, 1, z0, False)
    block(1, 1, 2, None, z0, True)

    def q_step(j, carry):
        z0 = pl.multiple_of((j >> 8) * 8, 8)
        for u in range(UNROLL_Q):
            a = 2 + j * UNROLL_Q + u
            block(a, None, a + 1 if u + 1 < UNROLL_Q else jnp.minimum(a + 1, NQ - 1), None, z0, True)
        return carry

    lax.fori_loop(0, (NQ - 2) // UNROLL_Q, q_step, 0)
    out_proj(NQ - 1, pltpu.bitcast(o_s[...], bf16))
    for a in range(NQ):
        out_copy(a).wait()


@jax.jit
def pallas_parallel_sum__sliding_block__moe_arch_mod__prompt_kernel(
    A_x, A_wqkv, A_wo, B_x, B_w_r, B_w_gate, B_w_up, B_w_down,
):
    any_spec = pl.BlockSpec(memory_space=pl.ANY)
    out = pl.pallas_call(
        _kernel,
        out_shape=jax.ShapeDtypeStruct((SEQ, D), bf16),
        in_specs=[any_spec] * 7,
        out_specs=any_spec,
        scratch_shapes=[
            pltpu.VMEM((SEQ, D), bf16),
            pltpu.VMEM((D, 3 * D), bf16),
            pltpu.VMEM((D, D), bf16),
            pltpu.VMEM((D,), bf16),
            pltpu.VMEM((FF, D), bf16),
            pltpu.VMEM((FF, D), bf16),
            pltpu.VMEM((FF, D), bf16),
            pltpu.VMEM((SEQ // 2, D), i32),
            pltpu.VMEM((SEQ, D), f32),
            pltpu.VMEM((8, D), f32),
            pltpu.VMEM((SEQ // 2, D), i32),
            pltpu.VMEM(((SEQ + PAD) // 2, D), i32),
            pltpu.VMEM((NT, 256, 128), i32),
            pltpu.VMEM((328, 512), f32),
            pltpu.VMEM((328, 512), f32),
            pltpu.VMEM((QB // 2, D), i32),
            pltpu.VMEM((NQ, QB, D), bf16),
            pltpu.SemaphoreType.DMA((NA,)),
            pltpu.SemaphoreType.DMA((3,)),
            pltpu.SemaphoreType.DMA((5,)),
            pltpu.SemaphoreType.DMA((NQ,)),
        ],
        compiler_params=pltpu.CompilerParams(vmem_limit_bytes=100 * 1024 * 1024),
    )(A_x.reshape(SEQ, D), A_wqkv, A_wo, B_w_r, B_w_gate.T, B_w_up.T, B_w_down)
    return out.reshape(1, SEQ, D)
```

```python
import functools
import math

import jax
import jax.numpy as jnp
from jax import lax
from jax.experimental import pallas as pl
from jax.experimental.pallas import tpu as pltpu

bf16 = jnp.bfloat16
f32 = jnp.float32
i32 = jnp.int32

SEQ, D, DH, WIN, FF = 2048, 512, 16, 256, 1376
TB = 256
NA = SEQ // TB
LNCH = 16
QB = 128
NQ = SEQ // QB
PAD = 256
NEG = -1e9
QSCALE = DH ** -0.5 * math.log2(math.e)
NT = (SEQ + PAD) // 128
GATES = [0, 4, 8]
UNROLL_A = True
EARLY_AT = []
ORDER = 'VKQ'
NT_DIMS = (((1,), (1,)), ((), ()))


def _rb(x):
    return x.astype(bf16).astype(f32)


def _zero_like_bits(x):
    return lax.shift_right_logical(lax.shift_right_logical(pltpu.bitcast(x, i32), 31), 1)


def _pack16(x):
    return pltpu.pack_elementwise([x[0:8], x[8:16]], packed_dtype=bf16)


def _kernel(x_hbm, wqkv_hbm, wo_hbm, wr_hbm, wg_hbm, wu_hbm, wd_hbm, out_hbm,
            x_v, wqkv_v, wo_v, wr_v, wg_v, wu_v, wd_v,
            xn_s, xp_s, res_s, wr_s, q_s, qt_s, k_s, vt_s, s0_s, s1_s, s2_s, s3_s, s4_s, s5_s, o_s, ot_s, out_v,
            sem_x, sem_w, sem_m, sem_o):
    def x_copy(i):
        rows = pl.ds(i * TB, TB)
        return pltpu.make_async_copy(x_hbm.at[rows, :], x_v.at[rows, :], sem_x.at[i])

    def w_copy(g):
        cols = pl.ds(D * g, D)
        return pltpu.make_async_copy(wqkv_hbm.at[:, cols], wqkv_v.at[:, cols], sem_w.at[g])

    wq_copy, wk_copy, wv_copy = w_copy(0), w_copy(1), w_copy(2)
    wr_copy = pltpu.make_async_copy(wr_hbm, wr_v, sem_m.at[0])
    wo_copy = pltpu.make_async_copy(wo_hbm, wo_v, sem_m.at[1])
    ffn_copies = [pltpu.make_async_copy(wg_hbm, wg_v, sem_m.at[2]),
                  pltpu.make_async_copy(wu_hbm, wu_v, sem_m.at[3]),
                  pltpu.make_async_copy(wd_hbm, wd_v, sem_m.at[4])]
    x_copy(0).start()
    x_copy(1).start()
    wr_copy.start()
    wv_copy.start()

    k_s[pl.ds(0, PAD // 2), :] = jnp.zeros((PAD // 2, D), i32)
    vt_s[0] = jnp.zeros((256, 128), i32)
    vt_s[1] = jnp.zeros((256, 128), i32)

    row16 = lax.broadcasted_iota(i32, (16, 128), 0)

    def layer_norm(i, best, gate):
        wr = wr_s[...][0:1]
        z = None
        for c in range(TB // LNCH):
            r0 = pl.multiple_of(i * TB + LNCH * c, LNCH)
            xf = x_v[pl.ds(r0, LNCH), :].astype(f32)
            m32 = jnp.sum(xf, axis=-1, keepdims=True) * (1.0 / D)
            if z is not None:
                m32 = pltpu.bitcast(pltpu.bitcast(m32, i32) | z, f32)
            cen = xf - m32
            v32 = jnp.sum(cen * cen, axis=-1, keepdims=True) * (1.0 / D)
            d = _rb(xf - _rb(m32))
            ve = _rb(_rb(v32) + _rb(jnp.float32(1e-5)))
            s = _rb(ve * lax.rsqrt(ve))
            r = pltpu.reciprocal(s, approx=True)
            inv = r * (2.0 - s * r)
            if gate:
                z = _zero_like_bits(inv)
            xn = (d * inv).astype(bf16)
            xn32 = xn.astype(f32)
            half = pl.ds(pl.multiple_of(r0 // 2, LNCH // 2), LNCH // 2)
            xn_s[half, :] = pltpu.bitcast(xn, i32)
            xp_s[half, :] = _pack16(xn32)
            res_s[pl.ds(r0, LNCH), :] = xf + xn32
            rr = _rb(jnp.sum(xn32 * wr, axis=-1, keepdims=True))
            rr = jnp.broadcast_to(jnp.where(rr != rr, -jnp.inf, rr), (LNCH, 128))
            upd = rr > best[0]
            best[0] = jnp.where(upd, rr, best[0])
            best[1] = jnp.where(upd, row16 + r0, best[1])
            yield

    def load_xn(ref, i):
        return pltpu.bitcast(ref[pl.ds(pl.multiple_of(i * (TB // 2), TB // 2), TB // 2), :], bf16)

    def load_block(i):
        return load_xn(xn_s, i), load_xn(xp_s, i)

    def project(work, ln, hook=lambda n: None, defer=None):
        def finish(i, j, d):
            cols = slice(128 * (j % 4), 128 * (j % 4) + 128)
            if j < 4:
                q_s[pl.ds(pl.multiple_of(i * TB, TB), TB), cols] = d * QSCALE
            elif j < 8:
                r0 = pl.multiple_of(i * (TB // 2) + PAD // 2, TB // 2)
                k_s[pl.ds(r0, TB // 2), cols] = pltpu.bitcast(d.astype(bf16), i32)
            else:
                for t in range(TB // 128):
                    vt = d[128 * t:128 * t + 128].T
                    vt_s[i * (TB // 128) + t + PAD // 128, pl.ds(64 * (j % 4), 64), :] = pltpu.bitcast(vt.astype(bf16), i32)

        for n, (i, xn, j) in enumerate(work):
            next(ln, None)
            d = jnp.dot(xn[1] if j >= 8 else xn[0], wqkv_v[:, 128 * j:128 * j + 128], preferred_element_type=f32)
            if defer is None:
                finish(i, j, d)
            else:
                defer.append(functools.partial(finish, i, j, d))
            hook(n)
        for _ in ln:
            pass

    V_COLS, K_COLS, Q_COLS = [8, 9, 10, 11], [4, 5, 6, 7], [0, 1, 2, 3]
    ALL_COLS = [c for g in ORDER for c in dict(V=V_COLS, K=K_COLS, Q=Q_COLS)[g]]
    QK_COLS = [c for c in ALL_COLS if c < 8]

    wr_copy.wait()
    wk_copy.start()
    wq_copy.start()
    x_copy(2).start()
    wr_s[...] = jnp.broadcast_to(wr_v[...].astype(f32).reshape(1, D), (8, D))
    best = [jnp.full((16, 128), -jnp.inf, f32), row16]
    for i in range(2):
        x_copy(i).wait()
        for _ in layer_norm(i, best, False):
            pass
    xn0, xn1 = load_block(0), load_block(1)
    wv_copy.wait()
    for i in range(3, NA):
        x_copy(i).start()
    v_stores = []
    project([(0, xn0, j) for j in V_COLS] + [(1, xn1, j) for j in V_COLS], iter(()), defer=v_stores)
    wk_copy.wait()
    wq_copy.wait()
    x_copy(2).wait()
    wo_copy.start()
    for c in ffn_copies:
        c.start()
    for store in v_stores:
        store()
    project([(0, xn0, j) for j in QK_COLS] + [(1, xn1, j) for j in QK_COLS],
            layer_norm(2, best, True))
    best = tuple(best)

    def phase_a(i, carry):
        best = list(carry[0])
        x_copy(i + 1).wait()
        xn = load_block(i)
        project([(i, xn, j) for j in ALL_COLS], layer_norm(i + 1, best, True))
        return tuple(best), (i >> 8)

    (best_v, best_i), zero = lax.fori_loop(2, NA - 1, phase_a, (best, 0), unroll=UNROLL_A)
    z0 = pl.multiple_of(zero * 8, 8)

    rmax = jnp.max(best_v, axis=0, keepdims=True)
    idx = jnp.min(jnp.where(best_v == rmax, best_i, SEQ), axis=0, keepdims=True)[0, 0]
    slab = pltpu.bitcast(xn_s[pl.ds(pl.multiple_of((idx >> 4) * 8, 8), 8), :], bf16).astype(f32)
    rowsel = lax.broadcasted_iota(i32, (16, D), 0) == (idx & 15)
    xsel = jnp.sum(jnp.where(rowsel, slab, 0.0), axis=0, keepdims=True)
    xsel16 = jnp.broadcast_to(xsel, (16, D)).astype(bf16)

    wo_copy.wait()
    for c in ffn_copies:
        c.wait()
    f_tiles = [(f0, min(128, FF - f0)) for f0 in range(0, FF, 128)]
    hmid = []
    y_parts = []

    def gate_up(n):
        if n < len(f_tiles):
            f0, fn = f_tiles[n]
            g = lax.dot_general(xsel16, wg_v[pl.ds(f0, fn), :], NT_DIMS, preferred_element_type=f32)
            u = lax.dot_general(xsel16, wu_v[pl.ds(f0, fn), :], NT_DIMS, preferred_element_type=f32)
            hmid.append((g * jax.nn.sigmoid(g) * u).astype(bf16))

    def down():
        n = len(y_parts)
        if n < len(hmid):
            f0, fn = f_tiles[n]
            y_parts.append(jnp.dot(hmid[n], wd_v[pl.ds(f0, fn), :], preferred_element_type=f32))

    lane16 = lax.broadcasted_iota(i32, (16, 128), 1)
    col_j = lane16 & 63
    lo64 = lax.broadcasted_iota(i32, (64, 128), 1) < 64
    lo8 = lo64[0:8]
    lo1 = lo64[0:1]
    s_refs = [s0_s, s1_s, s2_s, s3_s, s4_s, s5_s]

    def first_chunk(static_a, ab):
        if static_a is None:
            return 0
        return max(0, PAD - (QB * static_a + 64 * ab)) // 16

    def transpose_q(a):
        for hg in range(4):
            qt = q_s[pl.ds(pl.multiple_of(a * QB, QB), QB), 128 * hg:128 * hg + 128].T
            qt = jnp.concatenate([qt[r:r + 16] if (r // 16) % 2 == 0 else pltpu.roll(qt[r:r + 16], 64, 1)
                                  for r in range(0, 128, 16)], axis=0)
            qt_s[a, pl.ds(64 * hg, 64), :] = pltpu.bitcast(qt.astype(bf16), i32)

    class Scores:
        def __init__(self, a, static_a, hg, ab, z0, buf):
            self.a, self.hg, self.ab, self.z0, self.ref = a, hg, ab, z0, s_refs[buf + ab]
            self.c0 = first_chunk(static_a, ab)
            zero8 = jnp.zeros((8, 128), i32)
            cols = []
            for p in range(4):
                qe = qt_s[a, pl.ds(64 * hg + 16 * p, 8), :]
                qo = qt_s[a, pl.ds(64 * hg + 16 * p + 8, 8), :]
                if ab == 0:
                    qe, qo = jnp.where(lo8, qe, 0), jnp.where(lo8, 0, qo)
                else:
                    qe, qo = jnp.where(lo8, 0, qe), jnp.where(lo8, qo, 0)
                cols.append(jnp.concatenate([zero8] * (2 * p) + [qe, qo] + [zero8] * (6 - 2 * p), axis=0))
            self.w = pltpu.bitcast(jnp.concatenate(cols, axis=1), bf16)
            self.acc = [None] * 4

        def part(self, half):
            mid = (self.c0 + 20) // 2
            c_lo, c_hi = (self.c0, mid) if half == 0 else (mid, 20)
            krow = pl.multiple_of(64 * self.a + 32 * self.ab + 8 * c_lo, 8)
            kw = pltpu.bitcast(k_s[pl.ds(krow, 8 * (c_hi - c_lo)), 128 * self.hg:128 * self.hg + 128], bf16)
            st = jnp.dot(kw, self.w, preferred_element_type=f32)
            popped = []
            for c in range(c_lo, c_hi):
                for p in range(4):
                    x = st[16 * (c - c_lo):16 * (c - c_lo) + 16, 128 * p:128 * p + 128]
                    if p == 3:
                        popped.append(x[0:8])
                    if c < 4:
                        x = jnp.where(row16 + 16 * c > col_j, x, NEG)
                    elif c >= 16:
                        x = jnp.where(row16 + 16 * (c - 16) <= col_j, x, NEG)
                    self.acc[p] = x if self.acc[p] is None else jnp.maximum(self.acc[p], x)
                    self.ref[pl.ds(self.z0 + 16 * c, 16), 128 * p:128 * p + 128] = x
            if half == 1:
                for p in range(4):
                    m = jnp.max(self.acc[p], axis=0, keepdims=True)
                    self.ref[pl.ds(self.z0 + 320, 8), 128 * p:128 * p + 128] = jnp.broadcast_to(m, (8, 128))
            return popped

    class Softmax:
        def __init__(self, static_a, hg, z0, buf):
            self.static_a, self.hg, self.z0, self.buf = static_a, hg, z0, buf
            self.tiles, self.acc, self.m = {}, {}, {}

        def tile(self, p, t, gate):
            for ab in range(2):
                if (ab, p, t) in self.tiles:
                    continue
                s_ref = s_refs[self.buf + ab]
                c0 = first_chunk(self.static_a, ab)
                if (ab, p) not in self.m:
                    self.m[ab, p] = s_ref[pl.ds(self.z0 + 320, 8), 128 * p:128 * p + 128]
                m = self.m[ab, p]
                if gate is not None:
                    m = pltpu.bitcast(pltpu.bitcast(m, i32) | gate, f32)
                rows = []
                for r in range(8 * t, 8 * t + 8):
                    c = r - 4 * ab
                    if not c0 <= c < 20:
                        rows.append(jnp.zeros((8, 128), i32))
                        continue
                    x = s_ref[pl.ds(self.z0 + 16 * c, 16), 128 * p:128 * p + 128]
                    e0, e1 = jnp.exp2(x[0:8] - m), jnp.exp2(x[8:16] - m)
                    a0 = self.acc.get((ab, p))
                    self.acc[ab, p] = (e0 if a0 is None else a0 + e0) + e1
                    rows.append(pltpu.pack_elementwise([e0, e1], packed_dtype=bf16))
                self.tiles[ab, p, t] = jnp.concatenate(rows, axis=0)

        def sums(self):
            return {k: jnp.sum(v, axis=0, keepdims=True) for k, v in self.acc.items()}

    def pv(a, hg, sm, ots, h, t):
        p = h // 2
        pa, pb = sm.tiles[0, p, t], sm.tiles[1, p, t]
        pt = jnp.where(lo64, pb, pa) if h % 2 else jnp.where(lo64, pa, pb)
        vv = pltpu.bitcast(vt_s[a + t, pl.ds(64 * hg + 8 * h, 8), :], bf16)
        d = jnp.dot(vv, pltpu.bitcast(pt, bf16), preferred_element_type=f32)
        ots[h] = ots[h] + d if h in ots else d

    def attend_pair(a, static_a, hg, p, z0, buf, handles):
        sm = Softmax(static_a, hg, z0, buf)
        ots = {}
        for t in range(0 if static_a is None else max(0, 2 - static_a), 3):
            gate = None
            if static_a is None and handles is not None and GATES[t] < len(handles):
                gate = _zero_like_bits(handles[GATES[t]])
            sm.tile(p, t, gate)
            for h in (2 * p, 2 * p + 1):
                pv(a, hg, sm, ots, h, t)
        sums = sm.sums()
        rows = []
        for h in (2 * p, 2 * p + 1):
            la, lb = sums[0, p], sums[1, p]
            l = jnp.where(lo1, lb, la) if h % 2 else jnp.where(lo1, la, lb)
            rl = pltpu.reciprocal(l, approx=True)
            rows.append(ots[h] * (rl * (2.0 - l * rl)))
        ot_s[32 * p:32 * p + 32, :] = jnp.concatenate(rows, axis=0)
        if p == 3:
            t = ot_s[...].T
            tsw = jnp.concatenate([t[64:128], t[0:64]], axis=0)
            odd = ((lax.broadcasted_iota(i32, (128, 128), 1) >> 4) & 1) == 1
            o = jnp.where(odd, tsw, t).astype(bf16)
            o_s[:, 128 * hg:128 * hg + 128] = pltpu.bitcast(o, i32)

    y_cache = []

    def routed_row():
        if not y_cache:
            assert len(y_parts) == len(f_tiles)
            y = y_parts[0]
            for part in y_parts[1:]:
                y = y + part
            y_cache.append(y[0:1] * jax.nn.sigmoid(rmax[:, 0:1]))
        return y_cache[0]

    def out_copy(a):
        return pltpu.make_async_copy(out_v.at[a], out_hbm.at[pl.ds(pl.multiple_of(a * QB, QB), QB), :], sem_o.at[a])

    def out_proj(a, o):
        attn = jnp.dot(o, wo_v[...], preferred_element_type=f32)
        r0 = pl.multiple_of(a * QB, QB)
        rowid = lax.broadcasted_iota(i32, (QB, D), 0) + a * QB
        out = attn + res_s[pl.ds(r0, QB), :] + jnp.where(rowid == idx, routed_row(), 0.0)
        out_v[a] = out.astype(bf16)
        out_copy(a).start()

    handles = [None]

    def step(new, old, z0, hook=lambda: None):
        for p in range(4):
            if new is not None:
                if p % 2 == 0:
                    sc = Scores(*new[:3], p // 2, z0, new[3])
                popped = sc.part(p % 2)
            else:
                popped = None
            hook()
            if old is not None:
                attend_pair(*old[:3], p, z0, old[3], handles[0])
            handles[0] = popped

    def group(n, a=None):
        if not 0 <= n < 4 * NQ:
            return None
        return (n // 4 if a is None else a, n // 4 if n < 8 else None, n % 4, 2 * (n % 3))

    def block(a, n0, z0, hook=lambda: None):
        for hg in range(4):
            n = n0 + hg
            new = group(n + 1, a + 1 if hg == 3 else a)
            old = group(n - 1, a - 1 if hg == 0 else a)
            if hg == 0 and group(n + 4) is not None:
                transpose_q(a + 1)
            step(new, old, z0, hook)
            if hg == 0 and old is not None:
                o_prev = pltpu.bitcast(o_s[...], bf16)
            yield
        if n0 >= 4:
            out_proj(a - 1, o_prev)

    def early_blocks():
        transpose_q(0)
        step(group(0), None, z0)
        yield
        for a in range(3):
            yield from block(a, 4 * a, z0, down)

    early_work = early_blocks()

    def last_block_hook(n):
        gate_up(n)
        for _ in range(EARLY_AT.count(n)):
            next(early_work, None)

    project([(NA - 1, load_block(NA - 1), j) for j in ALL_COLS], iter(()), last_block_hook)
    for _ in early_work:
        pass

    assert len(y_parts) == len(f_tiles)

    def q_step(j, carry):
        z = pl.multiple_of((j >> 8) * 8, 8)
        handles[0] = None
        for u in range(3):
            for _ in block(3 + 3 * j + u, 12 + 4 * u, z):
                pass
        return carry

    lax.fori_loop(0, 4, q_step, 0)
    handles[0] = None
    for _ in block(NQ - 1, 4 * (NQ - 1), z0):
        pass
    step(None, group(4 * NQ - 1), z0)
    out_proj(NQ - 1, pltpu.bitcast(o_s[...], bf16))
    for a in range(NQ):
        out_copy(a).wait()


@jax.jit
def pallas_parallel_sum__sliding_block__moe_arch_mod__prompt_kernel(
    A_x, A_wqkv, A_wo, B_x, B_w_r, B_w_gate, B_w_up, B_w_down,
):
    any_spec = pl.BlockSpec(memory_space=pl.ANY)
    out = pl.pallas_call(
        _kernel,
        out_shape=jax.ShapeDtypeStruct((SEQ, D), bf16),
        in_specs=[any_spec] * 7,
        out_specs=any_spec,
        scratch_shapes=[
            pltpu.VMEM((SEQ, D), bf16),
            pltpu.VMEM((D, 3 * D), bf16),
            pltpu.VMEM((D, D), bf16),
            pltpu.VMEM((D,), bf16),
            pltpu.VMEM((FF, D), bf16),
            pltpu.VMEM((FF, D), bf16),
            pltpu.VMEM((FF, D), bf16),
            pltpu.VMEM((SEQ // 2, D), i32),
            pltpu.VMEM((SEQ // 2, D), i32),
            pltpu.VMEM((SEQ, D), f32),
            pltpu.VMEM((8, D), f32),
            pltpu.VMEM((SEQ, D), f32),
            pltpu.VMEM((NQ, 256, 128), i32),
            pltpu.VMEM(((SEQ + PAD) // 2, D), i32),
            pltpu.VMEM((NT, 256, 128), i32),
            pltpu.VMEM((328, 512), f32),
            pltpu.VMEM((328, 512), f32),
            pltpu.VMEM((328, 512), f32),
            pltpu.VMEM((328, 512), f32),
            pltpu.VMEM((328, 512), f32),
            pltpu.VMEM((328, 512), f32),
            pltpu.VMEM((QB // 2, D), i32),
            pltpu.VMEM((128, 128), f32),
            pltpu.VMEM((NQ, QB, D), bf16),
            pltpu.SemaphoreType.DMA((NA,)),
            pltpu.SemaphoreType.DMA((3,)),
            pltpu.SemaphoreType.DMA((5,)),
            pltpu.SemaphoreType.DMA((NQ,)),
        ],
        compiler_params=pltpu.CompilerParams(vmem_limit_bytes=100 * 1024 * 1024),
    )(A_x.reshape(SEQ, D), A_wqkv, A_wo, B_w_r, B_w_gate.T, B_w_up.T, B_w_down)
    return out.reshape(1, SEQ, D)
```

```python
import functools
import math

import jax
import jax.numpy as jnp
from jax import lax
from jax.experimental import pallas as pl
from jax.experimental.pallas import tpu as pltpu

bf16 = jnp.bfloat16
f32 = jnp.float32
i32 = jnp.int32

SEQ, D, DH, FF = 2048, 512, 16, 1376
TB = 256
NA = SEQ // TB
LNCH = 16
QB = 128
NQ = SEQ // QB
PAD = 256
NT = (SEQ + PAD) // 128
NEG = -1e9
QSCALE = DH ** -0.5 * math.log2(math.e)
UNROLL = 6
GATES = (0, 5, 9)
V_COLS, K_COLS, Q_COLS = (8, 9, 10, 11), (4, 5, 6, 7), (0, 1, 2, 3)
NT_DIMS = (((1,), (1,)), ((), ()))


def _rb(x):
    return x.astype(bf16).astype(f32)


def _zero_from(x):
    return lax.shift_right_logical(lax.shift_right_logical(pltpu.bitcast(x, i32), 31), 1)


def _after(x, zero):
    return pltpu.bitcast(pltpu.bitcast(x, i32) | zero, f32)


def _pack16(lo, hi):
    return pltpu.pack_elementwise([lo, hi], packed_dtype=bf16)


def _kernel(x_hbm, wqkv_hbm, wo_hbm, wr_hbm, wg_hbm, wu_hbm, wd_hbm, out_hbm,
            x_v, wqkv_v, wo_v, wr_v, wg_v, wu_v, wd_v,
            xn_s, xp_s, res_s, wr_s, q_s, qt_s, k_s, vt_s, o_s, ot_s, out_v,
            s0_s, s1_s, s2_s, s3_s, s4_s, s5_s,
            sem_x, sem_w, sem_m, sem_o):
    def x_copy(i):
        rows = pl.ds(i * TB, TB)
        return pltpu.make_async_copy(x_hbm.at[rows, :], x_v.at[rows, :], sem_x.at[i])

    def w_copy(g):
        cols = pl.ds(D * g, D)
        return pltpu.make_async_copy(wqkv_hbm.at[:, cols], wqkv_v.at[:, cols], sem_w.at[g])

    wq_copy, wk_copy, wv_copy = w_copy(0), w_copy(1), w_copy(2)
    wr_copy = pltpu.make_async_copy(wr_hbm, wr_v, sem_m.at[0])
    wo_copy = pltpu.make_async_copy(wo_hbm, wo_v, sem_m.at[1])
    ffn_copies = [pltpu.make_async_copy(wg_hbm, wg_v, sem_m.at[2]),
                  pltpu.make_async_copy(wu_hbm, wu_v, sem_m.at[3]),
                  pltpu.make_async_copy(wd_hbm, wd_v, sem_m.at[4])]
    x_copy(0).start()
    x_copy(1).start()
    wr_copy.start()
    wv_copy.start()

    k_s[pl.ds(0, PAD // 2), :] = jnp.zeros((PAD // 2, D), i32)
    for t in range(PAD // 128):
        vt_s[t] = jnp.zeros((256, 128), i32)

    row16 = lax.broadcasted_iota(i32, (16, 128), 0)

    def layer_norm(i, best, chained):
        wr = wr_s[...][0:1]
        zero = None
        for c in range(TB // LNCH):
            r0 = i * TB + LNCH * c
            xf = x_v[pl.ds(r0, LNCH), :].astype(f32)
            m32 = jnp.sum(xf, axis=-1, keepdims=True) * (1.0 / D)
            if zero is not None:
                m32 = _after(m32, zero)
            cen = xf - m32
            v32 = jnp.sum(cen * cen, axis=-1, keepdims=True) * (1.0 / D)
            d = _rb(xf - _rb(m32))
            ve = _rb(_rb(v32) + _rb(jnp.float32(1e-5)))
            sd = _rb(ve * lax.rsqrt(ve))
            rc = pltpu.reciprocal(sd, approx=True)
            inv = rc * (2.0 - sd * rc)
            if chained:
                zero = _zero_from(inv)
            xn = (d * inv).astype(bf16)
            xn32 = xn.astype(f32)
            half = pl.ds(r0 // 2, LNCH // 2)
            xn_s[half, :] = pltpu.bitcast(xn, i32)
            xp_s[half, :] = _pack16(xn32[0:8], xn32[8:16])
            res_s[pl.ds(r0, LNCH), :] = xf + xn32
            r = _rb(jnp.sum(xn32 * wr, axis=-1, keepdims=True))
            r = jnp.broadcast_to(jnp.where(r != r, -jnp.inf, r), (LNCH, 128))
            better = r > best[0]
            best[0] = jnp.where(better, r, best[0])
            best[1] = jnp.where(better, row16 + r0, best[1])
            yield

    def load_block(i):
        rows = pl.ds(i * (TB // 2), TB // 2)
        return pltpu.bitcast(xn_s[rows, :], bf16), pltpu.bitcast(xp_s[rows, :], bf16)

    def project(i, xn, cols, ln, hook=lambda: None, defer=None):
        def store(j, d):
            jj = j % 4
            if j in Q_COLS:
                q_s[pl.ds(i * TB, TB), 128 * jj:128 * jj + 128] = d * QSCALE
            elif j in K_COLS:
                k_s[pl.ds((i * TB + PAD) // 2, TB // 2), 128 * jj:128 * jj + 128] = pltpu.bitcast(d.astype(bf16), i32)
            else:
                for t in range(TB // 128):
                    vt = d[128 * t:128 * t + 128].T.astype(bf16)
                    vt_s[(i * TB + PAD) // 128 + t, pl.ds(64 * jj, 64), :] = pltpu.bitcast(vt, i32)

        for j in cols:
            next(ln, None)
            d = jnp.dot(xn[1] if j in V_COLS else xn[0], wqkv_v[:, 128 * j:128 * j + 128], preferred_element_type=f32)
            if defer is None:
                store(j, d)
            else:
                defer.append(functools.partial(store, j, d))
            hook()

    def drain(gen):
        for _ in gen:
            pass

    wr_copy.wait()
    wk_copy.start()
    x_copy(2).start()
    wr_s[...] = jnp.broadcast_to(wr_v[...].astype(f32).reshape(1, D), (8, D))
    best = [jnp.full((16, 128), -jnp.inf, f32), row16]
    x_copy(0).wait()
    wq_copy.start()
    drain(layer_norm(0, best, False))
    x_copy(1).wait()
    ln = layer_norm(1, best, False)
    for _ in range(4):
        next(ln)

    wv_copy.wait()
    for i in range(3, NA):
        x_copy(i).start()
    stores = []
    xn0 = load_block(0)
    project(0, xn0, V_COLS, ln, defer=stores)
    drain(ln)
    xn1 = load_block(1)
    project(1, xn1, V_COLS, ln, defer=stores)

    wk_copy.wait()
    x_copy(2).wait()
    for store in stores:
        store()
    stores = []
    ln = layer_norm(2, best, True)
    project(0, xn0, K_COLS, ln, defer=stores)
    project(1, xn1, K_COLS, ln, defer=stores)

    wq_copy.wait()
    wo_copy.start()
    for c in ffn_copies:
        c.start()
    for store in stores:
        store()
    project(0, xn0, Q_COLS, ln)
    project(1, xn1, Q_COLS, ln)
    drain(ln)

    for i in range(3, NA):
        x_copy(i).wait()
    for i in range(2, NA - 1):
        xn = load_block(i)
        ln = layer_norm(i + 1, best, True)
        project(i, xn, V_COLS + K_COLS + Q_COLS, ln)
        drain(ln)

    rmax = jnp.max(best[0], axis=0, keepdims=True)
    idx = jnp.min(jnp.where(best[0] == rmax, best[1], SEQ), axis=0, keepdims=True)[0, 0]
    slab = pltpu.bitcast(xn_s[pl.ds(pl.multiple_of((idx >> 4) * 8, 8), 8), :], bf16).astype(f32)
    xsel = jnp.sum(jnp.where(lax.broadcasted_iota(i32, (16, D), 0) == (idx & 15), slab, 0.0), axis=0, keepdims=True)
    xsel16 = jnp.broadcast_to(xsel, (16, D)).astype(bf16)

    wo_copy.wait()
    for c in ffn_copies:
        c.wait()
    f_tiles = [(f0, min(128, FF - f0)) for f0 in range(0, FF, 128)]
    hidden, y_parts, y_row = [], [], []

    def ffn_gate_up():
        if len(hidden) < len(f_tiles):
            f0, fn = f_tiles[len(hidden)]
            g = lax.dot_general(xsel16, wg_v[pl.ds(f0, fn), :], NT_DIMS, preferred_element_type=f32)
            u = lax.dot_general(xsel16, wu_v[pl.ds(f0, fn), :], NT_DIMS, preferred_element_type=f32)
            hidden.append((g * jax.nn.sigmoid(g) * u).astype(bf16))

    def ffn_down():
        if len(y_parts) < len(hidden):
            f0, fn = f_tiles[len(y_parts)]
            y_parts.append(jnp.dot(hidden[len(y_parts)], wd_v[pl.ds(f0, fn), :], preferred_element_type=f32))

    def routed_row():
        if not y_row:
            assert len(y_parts) == len(f_tiles)
            y_row.append(functools.reduce(jnp.add, y_parts)[0:1] * jax.nn.sigmoid(rmax[:, 0:1]))
        return y_row[0]

    project(NA - 1, load_block(NA - 1), V_COLS + K_COLS + Q_COLS, iter(()), ffn_gate_up)

    col_j = lax.broadcasted_iota(i32, (16, 128), 1) & 63
    lo64 = lax.broadcasted_iota(i32, (64, 128), 1) < 64
    lo8, lo1 = lo64[0:8], lo64[0:1]
    s_refs = [s0_s, s1_s, s2_s, s3_s, s4_s, s5_s]

    def first_chunk(a_static, ab):
        return 0 if a_static is None else max(0, PAD - (QB * a_static + 64 * ab)) // 16

    def transpose_q(a):
        for hg in range(4):
            qt = q_s[pl.ds(pl.multiple_of(a * QB, QB), QB), 128 * hg:128 * hg + 128].T
            qt = jnp.concatenate([qt[r:r + 16] if r % 32 == 0 else pltpu.roll(qt[r:r + 16], 64, 1)
                                  for r in range(0, 128, 16)], axis=0)
            qt_s[a, pl.ds(64 * hg, 64), :] = pltpu.bitcast(qt.astype(bf16), i32)

    def scores(grp, ab, z0):
        a, a_static, hg, buf = grp
        ref, c0 = s_refs[buf + ab], first_chunk(a_static, ab)
        zero8 = jnp.zeros((8, 128), i32)
        tiles = []
        for p in range(4):
            qe = qt_s[a, pl.ds(64 * hg + 16 * p, 8), :]
            qo = qt_s[a, pl.ds(64 * hg + 16 * p + 8, 8), :]
            if ab == 0:
                qe, qo = jnp.where(lo8, qe, 0), jnp.where(lo8, 0, qo)
            else:
                qe, qo = jnp.where(lo8, 0, qe), jnp.where(lo8, qo, 0)
            tiles.append(jnp.concatenate([zero8] * (2 * p) + [qe, qo] + [zero8] * (6 - 2 * p), axis=0))
        w = pltpu.bitcast(jnp.concatenate(tiles, axis=1), bf16)
        acc = [None] * 4
        mid = 20 if c0 >= 12 else (c0 + 20) // 2
        for c_lo, c_hi in ((c0, mid), (mid, 20)):
            handles = []
            if c_hi > c_lo:
                krow = pl.multiple_of(64 * a + 32 * ab + 8 * c_lo, 8)
                kw = pltpu.bitcast(k_s[pl.ds(krow, 8 * (c_hi - c_lo)), 128 * hg:128 * hg + 128], bf16)
                st = jnp.dot(kw, w, preferred_element_type=f32)
                for c in range(c_lo, c_hi):
                    for p in range(4):
                        x = st[16 * (c - c_lo):16 * (c - c_lo) + 16, 128 * p:128 * p + 128]
                        if p == 3:
                            handles.append(x[0:8])
                        if c < 4:
                            x = jnp.where(row16 + 16 * c > col_j, x, NEG)
                        elif c >= 16:
                            x = jnp.where(row16 + 16 * (c - 16) <= col_j, x, NEG)
                        acc[p] = x if acc[p] is None else jnp.maximum(acc[p], x)
                        ref[pl.ds(z0 + 16 * c, 16), 128 * p:128 * p + 128] = x
            if c_lo < c_hi == 20:
                for p in range(4):
                    m = jnp.max(acc[p], axis=0, keepdims=True)
                    ref[pl.ds(z0 + 320, 8), 128 * p:128 * p + 128] = jnp.broadcast_to(m, (8, 128))
            yield handles

    def attend_pair(grp, p, z0, handles):
        a, a_static, hg, buf = grp
        cols = slice(128 * p, 128 * p + 128)
        m = [s_refs[buf + ab][pl.ds(z0 + 320, 8), cols] for ab in range(2)]
        total = [None, None]
        out = [None, None]
        for t in range(0 if a_static is None else max(0, 2 - a_static), 3):
            gate = None
            if a_static is None and handles and GATES[t] < len(handles):
                gate = _zero_from(handles[GATES[t]])
            pt = []
            for ab in range(2):
                mm = m[ab] if gate is None else _after(m[ab], gate)
                rows = []
                for c in range(8 * t - 4 * ab, 8 * t + 8 - 4 * ab):
                    if not first_chunk(a_static, ab) <= c < 20:
                        rows.append(jnp.zeros((8, 128), i32))
                        continue
                    x = s_refs[buf + ab][pl.ds(z0 + 16 * c, 16), cols]
                    e0, e1 = jnp.exp2(x[0:8] - mm), jnp.exp2(x[8:16] - mm)
                    total[ab] = (e0 if total[ab] is None else total[ab] + e0) + e1
                    rows.append(_pack16(e0, e1))
                pt.append(jnp.concatenate(rows, axis=0))
            for odd in range(2):
                ph = jnp.where(lo64, pt[odd], pt[1 - odd])
                vh = pltpu.bitcast(vt_s[a + t, pl.ds(64 * hg + 16 * p + 8 * odd, 8), :], bf16)
                d = jnp.dot(vh, pltpu.bitcast(ph, bf16), preferred_element_type=f32)
                out[odd] = d if out[odd] is None else out[odd] + d
        l = [jnp.sum(v, axis=0, keepdims=True) for v in total]
        rows = []
        for odd in range(2):
            lh = jnp.where(lo1, l[odd], l[1 - odd])
            rc = pltpu.reciprocal(lh, approx=True)
            rows.append(out[odd] * (rc * (2.0 - lh * rc)))
        ot_s[32 * p:32 * p + 32, :] = jnp.concatenate(rows, axis=0)
        if p == 3:
            o = ot_s[...].T
            swapped = jnp.concatenate([o[64:128], o[0:64]], axis=0)
            odd_head = ((lax.broadcasted_iota(i32, (128, 128), 1) >> 4) & 1) == 1
            o_s[:, 128 * hg:128 * hg + 128] = pltpu.bitcast(jnp.where(odd_head, swapped, o).astype(bf16), i32)

    def out_proj(a, o):
        rows = pl.ds(pl.multiple_of(a * QB, QB), QB)
        token = lax.broadcasted_iota(i32, (QB, D), 0) + a * QB
        attn = jnp.dot(o, wo_v[...], preferred_element_type=f32)
        out_v[rows, :] = (attn + res_s[rows, :] + jnp.where(token == idx, routed_row(), 0.0)).astype(bf16)

    def out_copy(a, n, slot):
        rows = pl.ds(pl.multiple_of(a * QB, QB), n * QB)
        return pltpu.make_async_copy(out_v.at[rows, :], out_hbm.at[rows, :], sem_o.at[slot])

    class Pipeline:
        def __init__(self, z0, hook=lambda: None):
            self.z0, self.hook, self.handles = z0, hook, None

        @staticmethod
        def group(n, a):
            return (a, n // 4 if n < 8 else None, n % 4, 2 * (n % 3)) if 0 <= n < 4 * NQ else None

        def step(self, new, old):
            for p in range(4):
                handles = None
                if new is not None:
                    if p % 2 == 0:
                        parts = scores(new, p // 2, self.z0)
                    handles = next(parts)
                self.hook()
                if old is not None:
                    attend_pair(old, p, self.z0, self.handles)
                self.handles = handles

        def block(self, a, n0):
            for hg in range(4):
                n = n0 + hg
                if hg == 0 and n0 + 4 < 4 * NQ:
                    transpose_q(a + 1)
                self.step(self.group(n + 1, a + 1 if hg == 3 else a), self.group(n - 1, a - 1 if hg == 0 else a))
                if hg == 0 and n0 > 0:
                    o_prev = pltpu.bitcast(o_s[...], bf16)
            if n0 > 0:
                out_proj(a - 1, o_prev)

    pipe = Pipeline(0, ffn_down)
    transpose_q(0)
    pipe.step(pipe.group(0, 0), None)
    for a in range(3):
        pipe.block(a, 4 * a)
    out_copy(0, 2, 0).start()

    def loop_body(j, carry):
        pipe = Pipeline(pl.multiple_of((j >> 8) * 8, 8))
        for u in range(UNROLL):
            pipe.block(3 + UNROLL * j + u, 12 + 4 * u)
            if u % 3 == 2:
                out_copy(UNROLL * j + u, 3, 1 + (UNROLL // 3) * j + u // 3).start()
        return carry

    lax.fori_loop(0, (NQ - 4) // UNROLL, loop_body, 0)
    pipe = Pipeline(0)
    pipe.block(NQ - 1, 4 * (NQ - 1))
    out_copy(NQ - 2, 1, 5).start()
    pipe.step(None, pipe.group(4 * NQ - 1, NQ - 1))
    out_proj(NQ - 1, pltpu.bitcast(o_s[...], bf16))
    out_copy(NQ - 1, 1, 6).start()

    out_copy(0, 2, 0).wait()
    for j in range(4):
        out_copy(2 + 3 * j, 3, 1 + j).wait()
    out_copy(NQ - 2, 1, 5).wait()
    out_copy(NQ - 1, 1, 6).wait()


@jax.jit
def pallas_parallel_sum__sliding_block__moe_arch_mod__prompt_kernel(
    A_x, A_wqkv, A_wo, B_x, B_w_r, B_w_gate, B_w_up, B_w_down,
):
    del B_x
    hbm = pl.BlockSpec(memory_space=pl.ANY)
    out = pl.pallas_call(
        _kernel,
        out_shape=jax.ShapeDtypeStruct((SEQ, D), bf16),
        in_specs=[hbm] * 7,
        out_specs=hbm,
        scratch_shapes=[
            pltpu.VMEM((SEQ, D), bf16),
            pltpu.VMEM((D, 3 * D), bf16),
            pltpu.VMEM((D, D), bf16),
            pltpu.VMEM((D,), bf16),
            pltpu.VMEM((FF, D), bf16),
            pltpu.VMEM((FF, D), bf16),
            pltpu.VMEM((FF, D), bf16),
            pltpu.VMEM((SEQ // 2, D), i32),
            pltpu.VMEM((SEQ // 2, D), i32),
            pltpu.VMEM((SEQ, D), f32),
            pltpu.VMEM((8, D), f32),
            pltpu.VMEM((SEQ, D), f32),
            pltpu.VMEM((NQ, 256, 128), i32),
            pltpu.VMEM(((SEQ + PAD) // 2, D), i32),
            pltpu.VMEM((NT, 256, 128), i32),
            pltpu.VMEM((QB // 2, D), i32),
            pltpu.VMEM((128, 128), f32),
            pltpu.VMEM((SEQ, D), bf16),
            *[pltpu.VMEM((328, 512), f32)] * 6,
            pltpu.SemaphoreType.DMA((NA,)),
            pltpu.SemaphoreType.DMA((3,)),
            pltpu.SemaphoreType.DMA((5,)),
            pltpu.SemaphoreType.DMA((7,)),
        ],
        compiler_params=pltpu.CompilerParams(vmem_limit_bytes=64 * 1024 * 1024),
    )(A_x.reshape(SEQ, D), A_wqkv, A_wo, B_w_r, B_w_gate.T, B_w_up.T, B_w_down)
    return out.reshape(1, SEQ, D)
```

```python
import functools
import math

import jax
import jax.numpy as jnp
from jax import lax
from jax.experimental import pallas as pl
from jax.experimental.pallas import tpu as pltpu

bf16 = jnp.bfloat16
f32 = jnp.float32
i32 = jnp.int32

SEQ, D, DH, FF = 2048, 512, 16, 1376
TB = 256
NA = SEQ // TB
LNCH = 16
QB = 128
NQ = SEQ // QB
PAD = 256
NT = (SEQ + PAD) // 128
NEG = -1e9
QSCALE = DH ** -0.5 * math.log2(math.e)
UNROLL = 6
XSPLIT = 6
GATES = (0, 5, 9)
V_COLS, K_COLS, Q_COLS = (8, 9, 10, 11), (4, 5, 6, 7), (0, 1, 2, 3)
NT_DIMS = (((1,), (1,)), ((), ()))


def _rb(x):
    return x.astype(bf16).astype(f32)


def _zero_from(x):
    return lax.shift_right_logical(lax.shift_right_logical(pltpu.bitcast(x, i32), 31), 1)


def _after(x, zero):
    return pltpu.bitcast(pltpu.bitcast(x, i32) | zero, f32)


def _pack16(lo, hi):
    return pltpu.pack_elementwise([lo, hi], packed_dtype=bf16)


def _kernel(x_hbm, wqkv_hbm, wo_hbm, wr_hbm, wg_hbm, wu_hbm, wd_hbm, out_hbm,
            x_v, wqkv_v, wo_v, wr_v, wg_v, wu_v, wd_v,
            xn_s, xp_s, res_s, wr_s, q_s, qt_s, k_s, vt_s, o_s, ot_s, out_v,
            s0_s, s1_s, s2_s, s3_s, s4_s, s5_s,
            sem_x, sem_w, sem_m, sem_o):
    def x_copy(i):
        rows = pl.ds(i * TB, TB)
        return pltpu.make_async_copy(x_hbm.at[rows, :], x_v.at[rows, :], sem_x.at[i])

    def w_copy(g):
        cols = pl.ds(D * g, D)
        return pltpu.make_async_copy(wqkv_hbm.at[:, cols], wqkv_v.at[:, cols], sem_w.at[g])

    wq_copy, wk_copy, wv_copy = w_copy(0), w_copy(1), w_copy(2)
    wr_copy = pltpu.make_async_copy(wr_hbm, wr_v, sem_m.at[0])
    wo_copy = pltpu.make_async_copy(wo_hbm, wo_v, sem_m.at[1])
    ffn_copies = [pltpu.make_async_copy(wg_hbm, wg_v, sem_m.at[2]),
                  pltpu.make_async_copy(wu_hbm, wu_v, sem_m.at[3]),
                  pltpu.make_async_copy(wd_hbm, wd_v, sem_m.at[4])]
    x_copy(0).start()
    x_copy(1).start()
    wr_copy.start()
    wv_copy.start()

    k_s[pl.ds(0, PAD // 2), :] = jnp.zeros((PAD // 2, D), i32)
    for t in range(PAD // 128):
        vt_s[t] = jnp.zeros((256, 128), i32)

    row16 = lax.broadcasted_iota(i32, (16, 128), 0)

    def layer_norm(i, best, chained):
        wr = wr_s[...][0:1]
        zero = None
        for c in range(TB // LNCH):
            r0 = i * TB + LNCH * c
            xf = x_v[pl.ds(r0, LNCH), :].astype(f32)
            m32 = jnp.sum(xf, axis=-1, keepdims=True) * (1.0 / D)
            if zero is not None:
                m32 = _after(m32, zero)
            cen = xf - m32
            v32 = jnp.sum(cen * cen, axis=-1, keepdims=True) * (1.0 / D)
            d = _rb(xf - _rb(m32))
            ve = _rb(_rb(v32) + _rb(jnp.float32(1e-5)))
            sd = _rb(ve * lax.rsqrt(ve))
            rc = pltpu.reciprocal(sd, approx=True)
            inv = rc * (2.0 - sd * rc)
            if chained:
                zero = _zero_from(inv)
            xn = (d * inv).astype(bf16)
            xn32 = xn.astype(f32)
            half = pl.ds(r0 // 2, LNCH // 2)
            xn_s[half, :] = pltpu.bitcast(xn, i32)
            xp_s[half, :] = _pack16(xn32[0:8], xn32[8:16])
            res_s[pl.ds(r0, LNCH), :] = xf + xn32
            r = _rb(jnp.sum(xn32 * wr, axis=-1, keepdims=True))
            r = jnp.broadcast_to(jnp.where(r != r, -jnp.inf, r), (LNCH, 128))
            better = r > best[0]
            best[0] = jnp.where(better, r, best[0])
            best[1] = jnp.where(better, row16 + r0, best[1])
            yield

    def load_block(i):
        rows = pl.ds(i * (TB // 2), TB // 2)
        return pltpu.bitcast(xn_s[rows, :], bf16), pltpu.bitcast(xp_s[rows, :], bf16)

    def project(i, xn, cols, ln, hook=lambda: None, defer=None):
        def store(j, d):
            jj = j % 4
            if j in Q_COLS:
                q_s[pl.ds(i * TB, TB), 128 * jj:128 * jj + 128] = d * QSCALE
            elif j in K_COLS:
                k_s[pl.ds((i * TB + PAD) // 2, TB // 2), 128 * jj:128 * jj + 128] = pltpu.bitcast(d.astype(bf16), i32)
            else:
                for t in range(TB // 128):
                    vt = d[128 * t:128 * t + 128].T.astype(bf16)
                    vt_s[(i * TB + PAD) // 128 + t, pl.ds(64 * jj, 64), :] = pltpu.bitcast(vt, i32)

        for j in cols:
            next(ln, None)
            d = jnp.dot(xn[1] if j in V_COLS else xn[0], wqkv_v[:, 128 * j:128 * j + 128], preferred_element_type=f32)
            if defer is None:
                store(j, d)
            else:
                defer.append(functools.partial(store, j, d))
            hook()

    def drain(gen):
        for _ in gen:
            pass

    wr_copy.wait()
    wk_copy.start()
    x_copy(2).start()
    wr_s[...] = jnp.broadcast_to(wr_v[...].astype(f32).reshape(1, D), (8, D))
    best = [jnp.full((16, 128), -jnp.inf, f32), row16]
    x_copy(0).wait()
    wq_copy.start()
    drain(layer_norm(0, best, False))
    x_copy(1).wait()
    ln = layer_norm(1, best, False)
    for _ in range(4):
        next(ln)

    wv_copy.wait()
    for i in range(3, XSPLIT):
        x_copy(i).start()
    stores = []
    xn0 = load_block(0)
    project(0, xn0, V_COLS, ln, defer=stores)
    drain(ln)
    xn1 = load_block(1)
    project(1, xn1, V_COLS, ln, defer=stores)

    wk_copy.wait()
    x_copy(2).wait()
    for store in stores:
        store()
    stores = []
    ln = layer_norm(2, best, True)
    project(0, xn0, K_COLS, ln, defer=stores)
    project(1, xn1, K_COLS, ln, defer=stores)

    wq_copy.wait()
    for i in range(3, XSPLIT):
        x_copy(i).wait()
    for i in range(XSPLIT, NA):
        x_copy(i).start()
    wo_copy.start()
    for c in ffn_copies:
        c.start()
    for store in stores:
        store()
    project(0, xn0, Q_COLS, ln)
    project(1, xn1, Q_COLS, ln)
    drain(ln)

    for i in range(2, NA - 1):
        if i == XSPLIT - 1:
            for c in [x_copy(k) for k in range(XSPLIT, NA)] + [wo_copy] + ffn_copies:
                c.wait()
        xn = load_block(i)
        ln = layer_norm(i + 1, best, True)
        project(i, xn, V_COLS + K_COLS + Q_COLS, ln)
        drain(ln)

    rmax = jnp.max(best[0], axis=0, keepdims=True)
    idx = jnp.min(jnp.where(best[0] == rmax, best[1], SEQ), axis=0, keepdims=True)[0, 0]
    slab = pltpu.bitcast(xn_s[pl.ds(pl.multiple_of((idx >> 4) * 8, 8), 8), :], bf16).astype(f32)
    xsel = jnp.sum(jnp.where(lax.broadcasted_iota(i32, (16, D), 0) == (idx & 15), slab, 0.0), axis=0, keepdims=True)
    xsel16 = jnp.broadcast_to(xsel, (16, D)).astype(bf16)

    f_tiles = [(f0, min(128, FF - f0)) for f0 in range(0, FF, 128)]
    hidden, y_parts, y_row = [], [], []

    def ffn_gate_up():
        if len(hidden) < len(f_tiles):
            f0, fn = f_tiles[len(hidden)]
            g = lax.dot_general(xsel16, wg_v[pl.ds(f0, fn), :], NT_DIMS, preferred_element_type=f32)
            u = lax.dot_general(xsel16, wu_v[pl.ds(f0, fn), :], NT_DIMS, preferred_element_type=f32)
            hidden.append((g * jax.nn.sigmoid(g) * u).astype(bf16))

    def ffn_down():
        if len(y_parts) < len(hidden):
            f0, fn = f_tiles[len(y_parts)]
            y_parts.append(jnp.dot(hidden[len(y_parts)], wd_v[pl.ds(f0, fn), :], preferred_element_type=f32))

    def routed_row():
        if not y_row:
            assert len(y_parts) == len(f_tiles)
            y_row.append(functools.reduce(jnp.add, y_parts)[0:1] * jax.nn.sigmoid(rmax[:, 0:1]))
        return y_row[0]

    project(NA - 1, load_block(NA - 1), V_COLS + K_COLS + Q_COLS, iter(()), ffn_gate_up)

    col_j = lax.broadcasted_iota(i32, (16, 128), 1) & 63
    lo64 = lax.broadcasted_iota(i32, (64, 128), 1) < 64
    lo8, lo1 = lo64[0:8], lo64[0:1]
    s_refs = [s0_s, s1_s, s2_s, s3_s, s4_s, s5_s]

    def first_chunk(a_static, ab):
        return 0 if a_static is None else max(0, PAD - (QB * a_static + 64 * ab)) // 16

    def transpose_q(a):
        for hg in range(4):
            qt = q_s[pl.ds(pl.multiple_of(a * QB, QB), QB), 128 * hg:128 * hg + 128].T
            qt = jnp.concatenate([qt[r:r + 16] if r % 32 == 0 else pltpu.roll(qt[r:r + 16], 64, 1)
                                  for r in range(0, 128, 16)], axis=0)
            qt_s[a, pl.ds(64 * hg, 64), :] = pltpu.bitcast(qt.astype(bf16), i32)

    def scores(grp, ab, z0):
        a, a_static, hg, buf = grp
        ref, c0 = s_refs[buf + ab], first_chunk(a_static, ab)
        zero8 = jnp.zeros((8, 128), i32)
        tiles = []
        for p in range(4):
            qe = qt_s[a, pl.ds(64 * hg + 16 * p, 8), :]
            qo = qt_s[a, pl.ds(64 * hg + 16 * p + 8, 8), :]
            if ab == 0:
                qe, qo = jnp.where(lo8, qe, 0), jnp.where(lo8, 0, qo)
            else:
                qe, qo = jnp.where(lo8, 0, qe), jnp.where(lo8, qo, 0)
            tiles.append(jnp.concatenate([zero8] * (2 * p) + [qe, qo] + [zero8] * (6 - 2 * p), axis=0))
        w = pltpu.bitcast(jnp.concatenate(tiles, axis=1), bf16)
        acc = [None] * 4
        mid = 20 if c0 >= 12 else (c0 + 20) // 2
        for c_lo, c_hi in ((c0, mid), (mid, 20)):
            handles = []
            if c_hi > c_lo:
                krow = pl.multiple_of(64 * a + 32 * ab + 8 * c_lo, 8)
                kw = pltpu.bitcast(k_s[pl.ds(krow, 8 * (c_hi - c_lo)), 128 * hg:128 * hg + 128], bf16)
                st = jnp.dot(kw, w, preferred_element_type=f32)
                for c in range(c_lo, c_hi):
                    for p in range(4):
                        x = st[16 * (c - c_lo):16 * (c - c_lo) + 16, 128 * p:128 * p + 128]
                        if p == 3:
                            handles.append(x[0:8])
                        if c < 4:
                            x = jnp.where(row16 + 16 * c > col_j, x, NEG)
                        elif c >= 16:
                            x = jnp.where(row16 + 16 * (c - 16) <= col_j, x, NEG)
                        acc[p] = x if acc[p] is None else jnp.maximum(acc[p], x)
                        ref[pl.ds(z0 + 16 * c, 16), 128 * p:128 * p + 128] = x
            if c_lo < c_hi == 20:
                for p in range(4):
                    m = jnp.max(acc[p], axis=0, keepdims=True)
                    ref[pl.ds(z0 + 320, 8), 128 * p:128 * p + 128] = jnp.broadcast_to(m, (8, 128))
            yield handles

    def attend_pair(grp, p, z0, handles):
        a, a_static, hg, buf = grp
        cols = slice(128 * p, 128 * p + 128)
        m = [s_refs[buf + ab][pl.ds(z0 + 320, 8), cols] for ab in range(2)]
        total = [None, None]
        out = [None, None]
        for t in range(0 if a_static is None else max(0, 2 - a_static), 3):
            gate = None
            if a_static is None and handles and GATES[t] < len(handles):
                gate = _zero_from(handles[GATES[t]])
            pt = []
            for ab in range(2):
                mm = m[ab] if gate is None else _after(m[ab], gate)
                rows = []
                for c in range(8 * t - 4 * ab, 8 * t + 8 - 4 * ab):
                    if not first_chunk(a_static, ab) <= c < 20:
                        rows.append(jnp.zeros((8, 128), i32))
                        continue
                    x = s_refs[buf + ab][pl.ds(z0 + 16 * c, 16), cols]
                    e0, e1 = jnp.exp2(x[0:8] - mm), jnp.exp2(x[8:16] - mm)
                    total[ab] = (e0 if total[ab] is None else total[ab] + e0) + e1
                    rows.append(_pack16(e0, e1))
                pt.append(jnp.concatenate(rows, axis=0))
            for odd in range(2):
                ph = jnp.where(lo64, pt[odd], pt[1 - odd])
                vh = pltpu.bitcast(vt_s[a + t, pl.ds(64 * hg + 16 * p + 8 * odd, 8), :], bf16)
                d = jnp.dot(vh, pltpu.bitcast(ph, bf16), preferred_element_type=f32)
                out[odd] = d if out[odd] is None else out[odd] + d
        l = [jnp.sum(v, axis=0, keepdims=True) for v in total]
        rows = []
        for odd in range(2):
            lh = jnp.where(lo1, l[odd], l[1 - odd])
            rc = pltpu.reciprocal(lh, approx=True)
            rows.append(out[odd] * (rc * (2.0 - lh * rc)))
        ot_s[32 * p:32 * p + 32, :] = jnp.concatenate(rows, axis=0)
        if p == 3:
            o = ot_s[...].T
            swapped = jnp.concatenate([o[64:128], o[0:64]], axis=0)
            odd_head = ((lax.broadcasted_iota(i32, (128, 128), 1) >> 4) & 1) == 1
            o_s[:, 128 * hg:128 * hg + 128] = pltpu.bitcast(jnp.where(odd_head, swapped, o).astype(bf16), i32)

    def out_proj(a, o):
        rows = pl.ds(pl.multiple_of(a * QB, QB), QB)
        token = lax.broadcasted_iota(i32, (QB, D), 0) + a * QB
        attn = jnp.dot(o, wo_v[...], preferred_element_type=f32)
        out_v[rows, :] = (attn + res_s[rows, :] + jnp.where(token == idx, routed_row(), 0.0)).astype(bf16)

    def out_copy(a, n, slot):
        rows = pl.ds(pl.multiple_of(a * QB, QB), n * QB)
        return pltpu.make_async_copy(out_v.at[rows, :], out_hbm.at[rows, :], sem_o.at[slot])

    class Pipeline:
        def __init__(self, z0, hook=lambda: None):
            self.z0, self.hook, self.handles = z0, hook, None

        @staticmethod
        def group(n, a):
            return (a, n // 4 if n < 8 else None, n % 4, 2 * (n % 3)) if 0 <= n < 4 * NQ else None

        def step(self, new, old):
            for p in range(4):
                handles = None
                if new is not None:
                    if p % 2 == 0:
                        parts = scores(new, p // 2, self.z0)
                    handles = next(parts)
                self.hook()
                if old is not None:
                    attend_pair(old, p, self.z0, self.handles)
                self.handles = handles

        def block(self, a, n0):
            for hg in range(4):
                n = n0 + hg
                if hg == 0 and n0 + 4 < 4 * NQ:
                    transpose_q(a + 1)
                self.step(self.group(n + 1, a + 1 if hg == 3 else a), self.group(n - 1, a - 1 if hg == 0 else a))
                if hg == 0 and n0 > 0:
                    o_prev = pltpu.bitcast(o_s[...], bf16)
            if n0 > 0:
                out_proj(a - 1, o_prev)

    pipe = Pipeline(0)
    transpose_q(0)
    pipe.step(pipe.group(0, 0), None)
    pipe.hook = ffn_down
    for a in range(3):
        pipe.block(a, 4 * a)
    out_copy(0, 2, 0).start()

    def loop_body(j, carry):
        pipe = Pipeline(pl.multiple_of((j >> 8) * 8, 8))
        for u in range(UNROLL):
            pipe.block(3 + UNROLL * j + u, 12 + 4 * u)
            if u % 3 == 2:
                out_copy(UNROLL * j + u, 3, 1 + (UNROLL // 3) * j + u // 3).start()
        return carry

    lax.fori_loop(0, (NQ - 4) // UNROLL, loop_body, 0)
    pipe = Pipeline(0)
    pipe.block(NQ - 1, 4 * (NQ - 1))
    out_copy(NQ - 2, 1, 5).start()
    pipe.step(None, pipe.group(4 * NQ - 1, NQ - 1))
    out_proj(NQ - 1, pltpu.bitcast(o_s[...], bf16))
    out_copy(NQ - 1, 1, 6).start()

    out_copy(0, 2, 0).wait()
    for j in range(4):
        out_copy(2 + 3 * j, 3, 1 + j).wait()
    out_copy(NQ - 2, 1, 5).wait()
    out_copy(NQ - 1, 1, 6).wait()


@jax.jit
def pallas_parallel_sum__sliding_block__moe_arch_mod__prompt_kernel(
    A_x, A_wqkv, A_wo, B_x, B_w_r, B_w_gate, B_w_up, B_w_down,
):
    del B_x
    hbm = pl.BlockSpec(memory_space=pl.ANY)
    out = pl.pallas_call(
        _kernel,
        out_shape=jax.ShapeDtypeStruct((SEQ, D), bf16),
        in_specs=[hbm] * 7,
        out_specs=hbm,
        scratch_shapes=[
            pltpu.VMEM((SEQ, D), bf16),
            pltpu.VMEM((D, 3 * D), bf16),
            pltpu.VMEM((D, D), bf16),
            pltpu.VMEM((D,), bf16),
            pltpu.VMEM((FF, D), bf16),
            pltpu.VMEM((FF, D), bf16),
            pltpu.VMEM((FF, D), bf16),
            pltpu.VMEM((SEQ // 2, D), i32),
            pltpu.VMEM((SEQ // 2, D), i32),
            pltpu.VMEM((SEQ, D), f32),
            pltpu.VMEM((8, D), f32),
            pltpu.VMEM((SEQ, D), f32),
            pltpu.VMEM((NQ, 256, 128), i32),
            pltpu.VMEM(((SEQ + PAD) // 2, D), i32),
            pltpu.VMEM((NT, 256, 128), i32),
            pltpu.VMEM((QB // 2, D), i32),
            pltpu.VMEM((128, 128), f32),
            pltpu.VMEM((SEQ, D), bf16),
            *[pltpu.VMEM((328, 512), f32)] * 6,
            pltpu.SemaphoreType.DMA((NA,)),
            pltpu.SemaphoreType.DMA((3,)),
            pltpu.SemaphoreType.DMA((5,)),
            pltpu.SemaphoreType.DMA((7,)),
        ],
        compiler_params=pltpu.CompilerParams(vmem_limit_bytes=64 * 1024 * 1024,
                                             flags={"XLA_TPU_EVENLY_DISTRIBUTE_CRITICAL_NODES": True}),
    )(A_x.reshape(SEQ, D), A_wqkv, A_wo, B_w_r, B_w_gate.T, B_w_up.T, B_w_down)
    return out.reshape(1, SEQ, D)
```
